```python
import os as _os
_os.environ.setdefault("JAX_PLATFORMS", "cpu")
import jax
import jax.numpy as jnp

def _softmax(x, axis=-1):
    return jax.nn.softmax(x, axis=axis)
def _gelu(x):
    return jax.nn.gelu(x, approximate=True)
def _silu(x):
    return jax.nn.silu(x)
def _sigmoid(x):
    return jax.nn.sigmoid(x)
def _layernorm(x, axis=-1, eps=1e-5):
    m = jnp.mean(x, axis=axis, keepdims=True)
    v = jnp.var(x, axis=axis, keepdims=True)
    return (x - m) / jnp.sqrt(v + eps)
def _scatter_add(tgt, idx, src, axis=0):
    return tgt.at[idx].add(src)
def _segment_sum(src, seg, n):
    return jax.ops.segment_sum(src, seg, n)
class _Rng:
    def __init__(self, key):
        self._k = key
    def _next(self):
        self._k, sub = jax.random.split(self._k)
        return sub
    def normal(self, shape):
        return jax.random.normal(self._next(), shape, dtype=jnp.bfloat16)
    def randint(self, lo, hi, shape):
        return jax.random.randint(self._next(), shape, lo, hi, dtype=jnp.int32)
    def uniform(self, shape, lo=0.0, hi=1.0):
        return jax.random.uniform(self._next(), shape, jnp.bfloat16, lo, hi)
    def permutation(self, n):
        return jax.random.permutation(self._next(), n)


kernel_name = 'gated_mix__linear_kernel_hedgehog__glu_gated_bilinear__prompt'

def setup_inputs():
    _rng = _Rng(jax.random.key(int.from_bytes(__import__("os").urandom(4), "little")))
    _w = (lambda a: (lambda t: t.astype(jnp.bfloat16) if jnp.issubdtype(t.dtype, jnp.floating) else t)(jnp.asarray(a)))
    def _A_setup():
        B, S, D, H = 1, 2048, 512, 32
        Dh = D // H
        return {
            "x": _w((lambda *s: _rng.normal(s) * 0.05)(B, S, D)),
            "wqkv": _w((lambda *s: _rng.normal(s) * 0.8)(D, 3 * D)),
            "w_phi": _w((lambda *s: _rng.normal(s) * 0.8)(H, Dh, Dh) * (Dh ** -0.5)),
            "wo": _w((lambda *s: _rng.normal(s) * 0.05)(D, D)),
        }
    _A_in = _A_setup()

    def _B_setup():
        B, S, D, F = 1, 2048, 512, 1792
        return {
            "x": _w((lambda *s: _rng.normal(s) * 0.05)(B, S, D)),
            "w_gate": _w((lambda *s: _rng.normal(s) * 1.6)(D, F) * (D ** -0.5)),
            "w_up": _w((lambda *s: _rng.normal(s) * 1.6)(D, F) * (D ** -0.5)),
            "w_down": _w((lambda *s: _rng.normal(s) * 1.6)(F, D) * (F ** -0.5)),
        }
    _B_in = _B_setup()

    return {
        "A_x": _A_in["x"],
        "A_wqkv": _A_in["wqkv"],
        "A_w_phi": _A_in["w_phi"],
        "A_wo": _A_in["wo"],
        "B_x": _B_in["x"],
        "B_w_gate": _B_in["w_gate"],
        "B_w_up": _B_in["w_up"],
        "B_w_down": _B_in["w_down"],
        "gate_w": _w((lambda *s: _rng.normal(s) * 0.05)(512) * 16.0),
    }

def reference(A_x, A_wqkv, A_w_phi, A_wo, B_x, B_w_gate, B_w_up, B_w_down, gate_w):
    def _A_ref(x, wqkv, w_phi, wo):
        B, S, D = x.shape
        H = 32; Dh = D // H
        qkv = (lambda x, *d: x.transpose(*d))((x @ wqkv).reshape(B, S, 3, H, Dh), 2, 0, 3, 1, 4)
        q, k, v = qkv[0], qkv[1], qkv[2]
        pq = jnp.einsum("bhsd,hdf->bhsf", q, w_phi)
        pk = jnp.einsum("bhsd,hdf->bhsf", k, w_phi)
        phi_q = jnp.concatenate([_softmax(pq, axis=-1), _softmax(-pq, axis=-1)], axis=-1)
        phi_k = jnp.concatenate([_softmax(pk, axis=-1), _softmax(-pk, axis=-1)], axis=-1)
        kv = jnp.einsum("bhsf,bhsd->bhfd", phi_k, v)
        z  = jnp.einsum("bhsf->bhf", phi_k)
        num = jnp.einsum("bhqf,bhfd->bhqd", phi_q, kv)
        den = jnp.einsum("bhqf,bhf->bhq", phi_q, z)[..., None] + 1e-6
        o = num / den
        return (lambda x, *d: x.transpose(*d))(o, 0, 2, 1, 3).reshape(B, S, D) @ wo

    def _B_ref(x, w_gate, w_up, w_down):
        g = jnp.einsum("bsd,df->bsf", x, w_gate)
        u = jnp.einsum("bsd,df->bsf", x, w_up)
        h = g * u
        return jnp.einsum("bsf,fd->bsd", h, w_down)

    x = A_x
    g = _sigmoid((x * gate_w).sum(-1, keepdims=True))
    a = _A_ref(x, A_wqkv, A_w_phi, A_wo)
    b = _B_ref(x, B_w_gate, B_w_up, B_w_down)
    return g * a + (1 - g) * b
```

```python
import functools
import jax
import jax.numpy as jnp
from jax import lax
import jax.experimental.pallas as pl
import jax.experimental.pallas.tpu as pltpu

S, D, H, DH, F = 2048, 512, 32, 16, 1792
NG = 4
GW = 128
NT_DIMS = (((1,), (1,)), ((), ()))
TN_DIMS = (((0,), (0,)), ((), ()))
f32 = jnp.float32
bf16 = jnp.bfloat16


def _exp_pair(pT, ts):
    p4 = pT.reshape(NG, DH, 8, ts)
    mx = jnp.max(p4, axis=1, keepdims=True)
    mn = jnp.min(p4, axis=1, keepdims=True)
    ep = jnp.exp(p4 - mx)
    en = jnp.exp(mn - p4)
    sp = jnp.sum(ep, axis=1, keepdims=True)
    sn = jnp.sum(en, axis=1, keepdims=True)
    return ep, en, sp, sn


def _iota(shape, dim):
    return lax.broadcasted_iota(jnp.int32, shape, dim)


def _kernel(x_hbm, wqkv_hbm, wphi_hbm, wo_hbm, wg_hbm, wu_hbm, wd_hbm, gw_hbm, o_ref,
            x_v, wq_v, wk_v, wv_v, wphi_v, wo_v, wg_v, wu_v, wd_v, gw_v,
            tmat, wqT, wkT, kv_acc, z_acc, kvT, zb, sems, xsems, *, ts, do1=True, do2=True):
    p = pl.program_id(0)
    i = pl.program_id(1)
    nt = S // ts
    nlb = ts // 128

    def cp(k):
        src, dst = [
            (wphi_hbm, wphi_v),
            (wqkv_hbm.at[:, D:2 * D], wk_v),
            (wqkv_hbm.at[:, 2 * D:3 * D], wv_v),
            (wqkv_hbm.at[:, 0:D], wq_v),
            (wg_hbm, wg_v), (wu_hbm, wu_v), (wd_hbm, wd_v), (wo_hbm, wo_v), (gw_hbm, gw_v),
        ][k]
        return pltpu.make_async_copy(src, dst, sems.at[k])

    def xcp(t):
        return pltpu.make_async_copy(x_hbm.at[pl.ds(t * ts, ts), :], x_v.at[pl.ds(t * ts, ts), :], xsems.at[t])

    @pl.when(jnp.logical_and(p == 0, i == 0))
    def _prep():
        cp(0).start()
        cp(1).start()
        xcp(0).start()
        cp(2).start()
        kv_acc[...] = jnp.zeros_like(kv_acc)
        z_acc[...] = jnp.zeros_like(z_acc)
        cmat = jnp.where(_iota((H, D), 0) == (_iota((H, D), 1) >> 4), 1.0, 0.0).astype(bf16)
        amat = jnp.where((_iota((GW, 256), 0) >> 3) == (_iota((GW, 256), 1) & 15), 1.0, 0.0).astype(bf16)
        m1 = (_iota((256, D), 0) >> 4) == (_iota((256, D), 1) & 15)
        m2 = (_iota((GW, D), 0) & 7) == ((_iota((GW, D), 1) >> 4) & 7)
        cp(0).wait()
        e = jnp.dot(wphi_v[...], cmat, preferred_element_type=f32)
        e = jnp.where(m1, e, 0.0).astype(bf16)
        t = jnp.dot(amat, e, preferred_element_type=f32)
        t = jnp.where(m2, t, 0.0).astype(bf16)
        tmat[...] = t
        cp(1).wait()
        for tt in range(1, nt):
            xcp(tt).start()
        for k in range(3, 9):
            cp(k).start()
        for g in range(NG):
            wkT[g * GW:(g + 1) * GW, :] = lax.dot_general(
                t[:, g * GW:(g + 1) * GW], wk_v[:, g * GW:(g + 1) * GW], NT_DIMS,
                preferred_element_type=f32).astype(bf16)
        cp(2).wait()

    @pl.when(p == 0)
    def _kside():
        xcp(i).wait()
        if not do1:
            return
        xt = x_v[pl.ds(pl.multiple_of(i * ts, ts), ts), :]
        pkT = lax.dot_general(wkT[...], xt, NT_DIMS, preferred_element_type=f32)
        v = jnp.dot(xt, wv_v[...], preferred_element_type=f32).astype(bf16)
        ep, en, sp, sn = _exp_pair(pkT, ts)
        php = ep * (1.0 / sp)
        phn = en * (1.0 / sn)
        for g in range(NG):
            ph = jnp.concatenate([php[g].reshape(GW, ts), phn[g].reshape(GW, ts)], axis=0)
            zs = ph[:, 0:128]
            for l in range(1, nlb):
                zs = zs + ph[:, l * 128:(l + 1) * 128]
            z_acc[g] += zs
            kv_acc[g] += jnp.dot(ph.astype(bf16), v[:, g * GW:(g + 1) * GW],
                                 preferred_element_type=f32)

    @pl.when(jnp.logical_and(p == 1, i == 0))
    def _fin():
        msk = (_iota((2 * GW, GW), 0) & 7) == (_iota((2 * GW, GW), 1) >> 4)
        for g in range(NG):
            kvm = jnp.where(msk, kv_acc[g], 0.0)
            kvT[g] = kvm.T.astype(bf16)
            zs = jnp.sum(z_acc[g], axis=-1, keepdims=True)
            zb[g] = jnp.broadcast_to(zs, (2 * GW, ts))
        cp(3).wait()
        for g in range(NG):
            wqT[g * GW:(g + 1) * GW, :] = lax.dot_general(
                tmat[:, g * GW:(g + 1) * GW], wq_v[:, g * GW:(g + 1) * GW], NT_DIMS,
                preferred_element_type=f32).astype(bf16)
        for k in range(4, 9):
            cp(k).wait()

    @pl.when(p == 1)
    def _qside():
        xt = x_v[pl.ds(pl.multiple_of(i * ts, ts), ts), :]
        if not do2:
            o_ref[...] = xt
            return
        pqT = lax.dot_general(wqT[...], xt, NT_DIMS, preferred_element_type=f32)
        ep, en, sp, sn = _exp_pair(pqT, ts)
        oTs = []
        for g in range(NG):
            zp = zb[g, 0:GW, :].reshape(DH, 8, ts)
            zn = zb[g, GW:2 * GW, :].reshape(DH, 8, ts)
            np_ = jnp.sum(ep[g] * zp, axis=0, keepdims=True)
            nn_ = jnp.sum(en[g] * zn, axis=0, keepdims=True)
            isp = 1.0 / sp[g]
            isn = 1.0 / sn[g]
            den = np_ * isp + nn_ * isn + 1e-6
            iden = 1.0 / den
            php = (ep[g] * (isp * iden)).reshape(GW, ts)
            phn = (en[g] * (isn * iden)).reshape(GW, ts)
            ph = jnp.concatenate([php, phn], axis=0).astype(bf16)
            oTs.append(jnp.dot(kvT[g], ph, preferred_element_type=f32).astype(bf16))
        oT = jnp.concatenate(oTs, axis=0)
        a = lax.dot_general(oT, wo_v[...], TN_DIMS, preferred_element_type=f32)
        gg = jnp.dot(xt, wg_v[...], preferred_element_type=f32)
        uu = jnp.dot(xt, wu_v[...], preferred_element_type=f32)
        h = (gg * uu).astype(bf16)
        b = jnp.dot(h, wd_v[...], preferred_element_type=f32)
        logit = jnp.sum(xt.astype(f32) * gw_v[...].astype(f32), axis=-1, keepdims=True)
        gate = 1.0 / (1.0 + jnp.exp(-logit))
        o_ref[...] = (b + gate * (a - b)).astype(o_ref.dtype)


def _make(ts=256, **kw):
    nt = S // ts

    def fn(A_x, A_wqkv, A_w_phi, A_wo, B_x, B_w_gate, B_w_up, B_w_down, gate_w):
        x = A_x.reshape(S, D)
        wphi = A_w_phi.transpose(1, 2, 0).reshape(DH * DH, H)
        anyspec = pl.BlockSpec(memory_space=pl.ANY)
        out = pl.pallas_call(
            functools.partial(_kernel, ts=ts, **kw),
            grid=(2, nt),
            in_specs=[anyspec] * 8,
            out_specs=pl.BlockSpec((ts, D), lambda p, i: (i * p, 0)),
            out_shape=jax.ShapeDtypeStruct((S, D), bf16),
            scratch_shapes=[
                pltpu.VMEM((S, D), bf16),
                pltpu.VMEM((D, D), bf16), pltpu.VMEM((D, D), bf16), pltpu.VMEM((D, D), bf16),
                pltpu.VMEM((DH * DH, H), bf16), pltpu.VMEM((D, D), bf16),
                pltpu.VMEM((D, F), bf16), pltpu.VMEM((D, F), bf16), pltpu.VMEM((F, D), bf16),
                pltpu.VMEM((D,), bf16),
                pltpu.VMEM((GW, D), bf16),
                pltpu.VMEM((D, D), bf16), pltpu.VMEM((D, D), bf16),
                pltpu.VMEM((NG, 2 * GW, GW), f32), pltpu.VMEM((NG, 2 * GW, GW), f32),
                pltpu.VMEM((NG, GW, 2 * GW), bf16), pltpu.VMEM((NG, 2 * GW, ts), f32),
                pltpu.SemaphoreType.DMA((9,)), pltpu.SemaphoreType.DMA((nt,)),
            ],
            compiler_params=pltpu.CompilerParams(
                dimension_semantics=("arbitrary", "arbitrary"),
                vmem_limit_bytes=100 * 1024 * 1024),
        )(x, A_wqkv, wphi, A_wo, B_w_gate, B_w_up, B_w_down, gate_w)
        return out.reshape(1, S, D)
    return fn


@jax.jit
def pallas_gated_mix__linear_kernel_hedgehog__glu_gated_bilinear__prompt_kernel(
    A_x: jax.Array,
    A_wqkv: jax.Array,
    A_w_phi: jax.Array,
    A_wo: jax.Array,
    B_x: jax.Array,
    B_w_gate: jax.Array,
    B_w_up: jax.Array,
    B_w_down: jax.Array,
    gate_w: jax.Array,
):
    return _make(256)(A_x, A_wqkv, A_w_phi, A_wo, B_x, B_w_gate, B_w_up, B_w_down, gate_w)
```

```python
import functools
import jax
import jax.numpy as jnp
from jax import lax
import jax.experimental.pallas as pl
import jax.experimental.pallas.tpu as pltpu

S, D, H, DH, F = 2048, 512, 32, 16, 1792
NG = 8
GR = 64
NT_DIMS = (((1,), (1,)), ((), ()))
f32 = jnp.float32
bf16 = jnp.bfloat16
LOG2E = 1.4426950408889634


def _iota(shape, dim):
    return lax.broadcasted_iota(jnp.int32, shape, dim)


def _fold2(a, op):
    return op(a, pltpu.roll(a, 4, 1))


def _exp_pair(pT):
    ng, ts = pT.shape[0] // GR, pT.shape[1]
    p4 = pT.reshape(ng, 8, 8, ts)
    mx = _fold2(jnp.max(p4, axis=1), jnp.maximum)
    mn = _fold2(jnp.min(p4, axis=1), jnp.minimum)
    ep = jnp.exp2(p4 - mx[:, None])
    en = jnp.exp2(mn[:, None] - p4)
    sp = _fold2(jnp.sum(ep, axis=1), jnp.add)
    sn = _fold2(jnp.sum(en, axis=1), jnp.add)
    return ep, en, sp, sn


def _kernel(x_hbm, wqkv_hbm, wphi_hbm, wo_hbm, wg_hbm, wu_hbm, wd_hbm, gw_hbm, o_hbm,
            x_v, wq_v, wk_v, wv_v, wphi_v, wo_v, wg_v, wu_v, wd_v, gw_v,
            wqT, wkT, kvm, zb, o_v, o_s, sems, xsems, osems,
            *, ta, tb, merge, t2, tl, order2):
    tc = S - ta - tb
    HD = D // 2

    def cp(k):
        src, dst = [
            (wphi_hbm, wphi_v),
            (wqkv_hbm.at[:, D:D + HD], wk_v.at[:, 0:HD]),
            (wqkv_hbm.at[:, D + HD:2 * D], wk_v.at[:, HD:D]),
            (wqkv_hbm.at[:, 2 * D:3 * D], wv_v),
            (wqkv_hbm.at[:, 0:D], wq_v),
            (wg_hbm, wg_v), (wu_hbm, wu_v), (wd_hbm, wd_v), (wo_hbm, wo_v), (gw_hbm, gw_v),
        ][k]
        return pltpu.make_async_copy(src, dst, sems.at[k])

    def xcp(t):
        r0, n = [(0, ta), (ta, tb), (ta + tb, tc)][t]
        return pltpu.make_async_copy(x_hbm.at[pl.ds(r0, n), :], x_v.at[pl.ds(r0, n), :], xsems.at[t])

    n2 = (S - tl) // t2

    def ocp(t):
        if isinstance(t, int) and t == n2:
            return pltpu.make_async_copy(o_v.at[pl.ds(S - tl, tl), :], o_hbm.at[pl.ds(S - tl, tl), :],
                                         osems.at[t])
        return pltpu.make_async_copy(o_v.at[pl.ds(t * t2, t2), :], o_hbm.at[pl.ds(t * t2, t2), :],
                                     osems.at[t])

    cp(0).start()
    cp(1).start()
    xcp(0).start()
    cp(2).start()

    cmat = jnp.where(_iota((H, D), 0) == (_iota((H, D), 1) >> 4), 1.0, 0.0).astype(bf16)
    amat = jnp.where(((_iota((128, 256), 0) >> 2) & 15) == (_iota((128, 256), 1) & 15), 1.0, 0.0).astype(bf16)
    m1 = (_iota((256, D), 0) >> 4) == (_iota((256, D), 1) & 15)
    r2 = _iota((128, D), 0)
    m2 = (((r2 >> 6) << 2) | (r2 & 3)) == ((_iota((128, D), 1) >> 4) & 7)
    cp(0).wait()
    cp(3).start()
    e = jnp.dot(wphi_v[...], cmat, preferred_element_type=f32)
    e = jnp.where(m1, e, 0.0).astype(bf16)
    t = jnp.dot(amat, e, preferred_element_type=f32)
    t = jnp.where(m2, t, 0.0).astype(bf16)

    def fold(w_ref, dst, g):
        dst[g * 128:(g + 1) * 128, :] = (lax.dot_general(
            t[:, g * 128:(g + 1) * 128], w_ref[:, g * 128:(g + 1) * 128], NT_DIMS,
            preferred_element_type=f32) * LOG2E).astype(bf16)

    def k_p(xt, r0=0, r1=D):
        return lax.dot_general(wkT[r0:r1, :], xt, NT_DIMS, preferred_element_type=f32)

    def k_phi(pkT):
        ng, ts = pkT.shape[0] // GR, pkT.shape[1]
        ep, en, sp, sn = _exp_pair(pkT)
        php = (ep * (1.0 / sp)[:, None]).reshape(ng, GR, ts)
        phn = (en * (1.0 / sn)[:, None]).reshape(ng, GR, ts)
        ph = jnp.concatenate([php, phn], axis=1)
        zs = ph[:, :, 0:128]
        for l in range(1, ts // 128):
            zs = zs + ph[:, :, l * 128:(l + 1) * 128]
        return ph.astype(bf16), zs

    def k_v(xt):
        v = jnp.dot(xt, wv_v[...], preferred_element_type=f32).astype(bf16)
        return v.T

    def k_kv(vT, ph):
        return [lax.dot_general(vT[g * GR:(g + 1) * GR, :], ph[g], NT_DIMS, preferred_element_type=f32)
                for g in range(NG)]

    def add_l(a, b):
        return [u + w for u, w in zip(a, b)]

    cp(1).wait()
    xcp(1).start()
    fold(wk_v, wkT, 0)
    fold(wk_v, wkT, 1)
    xcp(0).wait()
    xcp(2).start()
    xa = x_v[0:ta, :]
    pha0, zsa0 = k_phi(k_p(xa, 0, HD))
    cp(2).wait()
    for k in range(4, 10):
        cp(k).start()
    fold(wk_v, wkT, 2)
    fold(wk_v, wkT, 3)
    pha1, zsa1 = k_phi(k_p(xa, HD, D))
    pha = jnp.concatenate([pha0, pha1], axis=0)
    zs = jnp.concatenate([zsa0, zsa1], axis=0)
    cp(3).wait()
    if merge:
        xcp(1).wait()
    vTa = k_v(xa)
    if not merge:
        kv = k_kv(vTa, pha)
        xcp(1).wait()
    xb = x_v[ta:ta + tb, :]
    pkb = k_p(xb)
    if merge:
        kv = k_kv(vTa, pha)
    vTb = k_v(xb)
    phb, zsb = k_phi(pkb)
    zs = zs + zsb
    kv = add_l(kv, k_kv(vTb, phb))
    xcp(2).wait()
    cp(4).wait()
    xc = x_v[ta + tb:S, :]
    pkc = k_p(xc)
    vTc = k_v(xc)
    phc, zsc = k_phi(pkc)
    zs = zs + zsc
    for g in range(4):
        fold(wq_v, wqT, g)
    kv = add_l(kv, k_kv(vTc, phc))
    msk = (_iota((GR, 128), 0) >> 4) == (_iota((GR, 128), 1) & 3)
    for g in range(NG):
        zb[g] = jnp.broadcast_to(jnp.sum(zs[g], axis=-1, keepdims=True), (128, 128))
        kvm[g] = jnp.where(msk, kv[g], 0.0).astype(bf16)
    for k in range(5, 10):
        cp(k).wait()

    def qsub(r0, ts):
        xt = x_v[pl.ds(r0, ts), :]
        env = {}

        def s_p():
            env['pqT'] = lax.dot_general(wqT[...], xt, NT_DIMS, preferred_element_type=f32)

        def s_phi():
            ep, en, sp, sn = _exp_pair(env['pqT'])
            zz = zb[...]
            zz = jnp.concatenate([zz] * (ts // 128), axis=2) if ts > 128 else zz
            zp = zz[:, 0:GR, :].reshape(NG, 8, 8, ts)
            zn = zz[:, GR:2 * GR, :].reshape(NG, 8, 8, ts)
            isp = 1.0 / sp
            isn = 1.0 / sn
            np_ = jnp.sum(ep * zp, axis=1) * isp + jnp.sum(en * zn, axis=1) * isn
            den = _fold2(np_, jnp.add) + 1e-6
            iden = 1.0 / den
            php = (ep * (isp * iden)[:, None]).reshape(NG, GR, ts)
            phn = (en * (isn * iden)[:, None]).reshape(NG, GR, ts)
            env['ph'] = jnp.concatenate([php, phn], axis=1).astype(bf16)

        def s_o():
            ph = env['ph']
            env['oT'] = jnp.concatenate(
                [jnp.dot(kvm[g], ph[g], preferred_element_type=f32).astype(bf16) for g in range(NG)], axis=0)

        def s_a():
            o_s[0:ts, :] = env['oT'].T
            env['a'] = jnp.dot(o_s[0:ts, :], wo_v[...], preferred_element_type=f32)

        def s_g():
            env['gg'] = jnp.dot(xt, wg_v[...], preferred_element_type=f32)

        def s_u():
            uu = jnp.dot(xt, wu_v[...], preferred_element_type=f32)
            env['h'] = (env['gg'] * uu).astype(bf16)

        def s_d():
            env['b'] = jnp.dot(env['h'], wd_v[...], preferred_element_type=f32)

        def s_l():
            logit = jnp.sum(xt.astype(f32) * gw_v[...].astype(f32), axis=-1, keepdims=True)
            env['gate'] = 0.5 * jnp.tanh(0.5 * logit) + 0.5

        st = dict(p=s_p, f=s_phi, o=s_o, a=s_a, g=s_g, u=s_u, d=s_d, l=s_l)
        for ch in order2:
            st[ch]()
        a, b = env['a'], env['b']
        o_v[pl.ds(r0, ts), :] = (b + env['gate'] * (a - b)).astype(bf16)

    def qbody(i, c):
        qsub(pl.multiple_of(i * t2, 128), t2)
        ocp(i).start()
        return c
    lax.fori_loop(0, n2, qbody, 0)
    if tl:
        qsub(S - tl, tl)
        ocp(n2).start()
    for tt in range(n2 + (1 if tl else 0)):
        ocp(tt).wait()


def _make(ta=256, tb=640, merge=False, t2=640, tl=128, order2='pgfuloda'):

    def fn(A_x, A_wqkv, A_w_phi, A_wo, B_x, B_w_gate, B_w_up, B_w_down, gate_w):
        x = A_x.reshape(S, D)
        wphi = A_w_phi.transpose(1, 2, 0).reshape(DH * DH, H)
        anyspec = pl.BlockSpec(memory_space=pl.ANY)
        out = pl.pallas_call(
            functools.partial(_kernel, ta=ta, tb=tb, merge=merge, t2=t2, tl=tl, order2=order2),
            in_specs=[anyspec] * 8,
            out_specs=anyspec,
            out_shape=jax.ShapeDtypeStruct((S, D), bf16),
            scratch_shapes=[
                pltpu.VMEM((S, D), bf16),
                pltpu.VMEM((D, D), bf16), pltpu.VMEM((D, D), bf16), pltpu.VMEM((D, D), bf16),
                pltpu.VMEM((DH * DH, H), bf16), pltpu.VMEM((D, D), bf16),
                pltpu.VMEM((D, F), bf16), pltpu.VMEM((D, F), bf16), pltpu.VMEM((F, D), bf16),
                pltpu.VMEM((D,), bf16),
                pltpu.VMEM((D, D), bf16), pltpu.VMEM((D, D), bf16),
                pltpu.VMEM((NG, GR, 128), bf16), pltpu.VMEM((NG, 128, 128), f32),
                pltpu.VMEM((S, D), bf16), pltpu.VMEM((t2, D), bf16),
                pltpu.SemaphoreType.DMA((10,)), pltpu.SemaphoreType.DMA((3,)),
                pltpu.SemaphoreType.DMA(((S - tl) // t2 + 1,)),
            ],
            compiler_params=pltpu.CompilerParams(vmem_limit_bytes=100 * 1024 * 1024),
        )(x, A_wqkv, wphi, A_wo, B_w_gate, B_w_up, B_w_down, gate_w)
        return out.reshape(1, S, D)
    return fn


@jax.jit
def pallas_gated_mix__linear_kernel_hedgehog__glu_gated_bilinear__prompt_kernel(
    A_x: jax.Array,
    A_wqkv: jax.Array,
    A_w_phi: jax.Array,
    A_wo: jax.Array,
    B_x: jax.Array,
    B_w_gate: jax.Array,
    B_w_up: jax.Array,
    B_w_down: jax.Array,
    gate_w: jax.Array,
):
    return _make(ta=384, tb=256, merge=True, t2=640, tl=128, order2='gpufloda')(A_x, A_wqkv, A_w_phi, A_wo, B_x, B_w_gate, B_w_up, B_w_down, gate_w)
```

```python
import jax
import jax.numpy as jnp
from jax import lax
import jax.experimental.pallas as pl
import jax.experimental.pallas.tpu as pltpu

S, D, H, DH, F = 2048, 512, 32, 16, 1792
HD, HF = D // 2, F // 2
NG = 8
GR = 64
TA, TB = 384, 384
TQ = 512
NQ = S // TQ
HQ = TQ // 2
NT_DIMS = (((1,), (1,)), ((), ()))
f32 = jnp.float32
bf16 = jnp.bfloat16
LOG2E = 1.4426950408889634


def _iota(shape, dim):
    return lax.broadcasted_iota(jnp.int32, shape, dim)


def _dot(a, b):
    return jnp.dot(a, b, preferred_element_type=f32)


def _dot_nt(a, b):
    return lax.dot_general(a, b, NT_DIMS, preferred_element_type=f32)


def _fold2(a, op):
    return op(a, pltpu.roll(a, 4, 1))


def _exp_pair(pT):
    ng, ts = pT.shape[0] // GR, pT.shape[1]
    p4 = pT.reshape(ng, 8, 8, ts)
    mx = _fold2(jnp.max(p4, axis=1), jnp.maximum)
    mn = _fold2(jnp.min(p4, axis=1), jnp.minimum)
    ep = jnp.exp2(p4 - mx[:, None])
    en = jnp.exp2(mn[:, None] - p4)
    sp = _fold2(jnp.sum(ep, axis=1), jnp.add)
    sn = _fold2(jnp.sum(en, axis=1), jnp.add)
    return ep, en, sp, sn


def _lhs_blocks(a11, a12, a21, a22):
    return [(a11 + a22).astype(bf16), (a21 + a22).astype(bf16), a11.astype(bf16), a22.astype(bf16),
            (a11 + a12).astype(bf16), (a21 - a11).astype(bf16), (a12 - a22).astype(bf16)]


def _rhs_blocks(w_ref, c0, c1):
    hk, hn = w_ref.shape[0] // 2, w_ref.shape[1] // 2
    b11, b12 = w_ref[:hk, c0:c1], w_ref[:hk, hn + c0:hn + c1]
    b21, b22 = w_ref[hk:, c0:c1], w_ref[hk:, hn + c0:hn + c1]
    f = lambda b: b.astype(f32)
    return [(f(b11) + f(b22)).astype(bf16), b11, (f(b12) - f(b22)).astype(bf16), (f(b21) - f(b11)).astype(bf16),
            b22, (f(b11) + f(b12)).astype(bf16), (f(b21) + f(b22)).astype(bf16)]


def _strassen(lhs, rhs):
    m = [_dot(lhs[i], rhs[i]) for i in range(7)]
    return (m[0] + m[3] - m[4] + m[6], m[2] + m[4], m[1] + m[3], m[0] - m[1] + m[2] + m[5])


def _block(c):
    return jnp.concatenate([jnp.concatenate([c[0], c[1]], axis=1),
                            jnp.concatenate([c[2], c[3]], axis=1)], axis=0)


def _kernel(x_hbm, wqkv_hbm, wphi_hbm, wo_hbm, wg_hbm, wu_hbm, wd_hbm, gw_hbm, o_hbm,
            x_v, wq_v, wk_v, wv_v, wphi_v, wo_v, wg_v, wu_v, wd_v, gw_v,
            wqT, wkT, kvm, zb, o_v, o_s, sems, xsems, osems):

    def cp(k):
        src, dst = [
            (wphi_hbm, wphi_v),
            (wqkv_hbm.at[:, D:D + HD], wk_v.at[:, 0:HD]),
            (wqkv_hbm.at[:, D + HD:2 * D], wk_v.at[:, HD:D]),
            (wqkv_hbm.at[:, 2 * D:3 * D], wv_v),
            (wqkv_hbm.at[:, 0:D], wq_v),
            (wg_hbm, wg_v), (wu_hbm, wu_v), (wd_hbm, wd_v), (wo_hbm, wo_v), (gw_hbm, gw_v),
        ][k]
        return pltpu.make_async_copy(src, dst, sems.at[k])

    def xcp(t):
        r0, n = [(0, TA), (TA, TB), (TA + TB, S - TA - TB)][t]
        return pltpu.make_async_copy(x_hbm.at[pl.ds(r0, n), :], x_v.at[pl.ds(r0, n), :], xsems.at[t])

    def ocp(i):
        r0 = i * TQ if isinstance(i, int) else pl.multiple_of(i * TQ, TQ)
        return pltpu.make_async_copy(o_v.at[pl.ds(r0, TQ), :], o_hbm.at[pl.ds(r0, TQ), :], osems.at[i])

    cp(0).start()
    cp(1).start()
    xcp(0).start()
    cp(2).start()

    cmat = jnp.where(_iota((H, D), 0) == (_iota((H, D), 1) >> 4), 1.0, 0.0).astype(bf16)
    amat = jnp.where(((_iota((128, 256), 0) >> 2) & 15) == (_iota((128, 256), 1) & 15), 1.0, 0.0).astype(bf16)
    m1 = (_iota((256, D), 0) >> 4) == (_iota((256, D), 1) & 15)
    r2 = _iota((128, D), 0)
    m2 = (((r2 >> 6) << 2) | (r2 & 3)) == ((_iota((128, D), 1) >> 4) & 7)
    cp(0).wait()
    cp(3).start()
    e = _dot(wphi_v[...], cmat)
    e = jnp.where(m1, e, 0.0).astype(bf16)
    t = _dot(amat, e)
    t = jnp.where(m2, t, 0.0).astype(bf16)

    def fold(w_ref, dst, g):
        w = _dot_nt(t[:, g * 128:(g + 1) * 128], w_ref[:, g * 128:(g + 1) * 128]) * LOG2E
        dst[g * 128:(g + 1) * 128, :] = w.astype(bf16)

    def k_phi(pkT):
        ts = pkT.shape[1]
        ep, en, sp, sn = _exp_pair(pkT)
        php = (ep * (1.0 / sp)[:, None]).reshape(NG, GR, ts)
        phn = (en * (1.0 / sn)[:, None]).reshape(NG, GR, ts)
        ph = jnp.concatenate([php, phn], axis=1)
        zs = ph[:, :, 0:128]
        for l in range(1, ts // 128):
            zs = zs + ph[:, :, l * 128:(l + 1) * 128]
        return ph.astype(bf16), zs

    def k_vT(xt):
        return _dot(xt, wv_v[...]).astype(bf16).T

    def k_kv(vT, ph):
        return [_dot_nt(vT[g * GR:(g + 1) * GR, :], ph[g]) for g in range(NG)]

    def add_l(a, b):
        return [u + w for u, w in zip(a, b)]

    cp(1).wait()
    xcp(1).start()
    fold(wk_v, wkT, 0)
    fold(wk_v, wkT, 1)
    xcp(0).wait()
    xcp(2).start()
    xa = x_v[0:TA, :]
    pka0 = _dot_nt(wkT[0:HD, :], xa)
    cp(2).wait()
    for k in range(4, 10):
        cp(k).start()
    fold(wk_v, wkT, 2)
    fold(wk_v, wkT, 3)
    pka1 = _dot_nt(wkT[HD:D, :], xa)
    cp(3).wait()
    xcp(1).wait()
    xb = x_v[TA:TA + TB, :]
    vTa = k_vT(xa)
    pha, zs = k_phi(jnp.concatenate([pka0, pka1], axis=0))
    pkb = _dot_nt(wkT[...], xb)
    vTb = k_vT(xb)
    kv = k_kv(vTa, pha)
    phb, zsb = k_phi(pkb)
    zs = zs + zsb
    kv = add_l(kv, k_kv(vTb, phb))
    xcp(2).wait()
    cp(4).wait()
    xc = x_v[TA + TB:S, :]
    pkc = _dot_nt(wkT[...], xc)
    vTc = k_vT(xc)
    phc, zsc = k_phi(pkc)
    zs = zs + zsc
    for g in range(4):
        fold(wq_v, wqT, g)
    kv = add_l(kv, k_kv(vTc, phc))
    msk = (_iota((GR, 128), 0) >> 4) == (_iota((GR, 128), 1) & 3)
    for g in range(NG):
        zb[g] = jnp.broadcast_to(jnp.sum(zs[g], axis=-1, keepdims=True), (128, 128))
        kvm[g] = jnp.where(msk, kv[g], 0.0).astype(bf16)
    for k in range(5, 10):
        cp(k).wait()

    def qbody(i, carry):
        r0 = pl.multiple_of(i * TQ, TQ)
        xt = x_v[pl.ds(r0, TQ), :]
        xf = xt.astype(f32)
        tx = _lhs_blocks(xf[:HQ, :HD], xf[:HQ, HD:], xf[HQ:, :HD], xf[HQ:, HD:])
        hs = []

        def gate_up(n):
            gg = _strassen(tx, _rhs_blocks(wg_v, n * 128, (n + 1) * 128))
            uu = _strassen(tx, _rhs_blocks(wu_v, n * 128, (n + 1) * 128))
            hs.append(_lhs_blocks(*[g_ * u_ for g_, u_ in zip(gg, uu)]))

        for n in range(0, 4):
            gate_up(n)
        pqT = _dot_nt(wqT[...], xt)
        for n in range(4, HF // 128):
            gate_up(n)

        ep, en, sp, sn = _exp_pair(pqT)
        zz = jnp.concatenate([zb[...]] * (TQ // 128), axis=2)
        zp = zz[:, 0:GR, :].reshape(NG, 8, 8, TQ)
        zn = zz[:, GR:2 * GR, :].reshape(NG, 8, 8, TQ)
        isp = 1.0 / sp
        isn = 1.0 / sn
        den = _fold2(jnp.sum(ep * zp, axis=1) * isp + jnp.sum(en * zn, axis=1) * isn, jnp.add) + 1e-6
        iden = 1.0 / den
        php = (ep * (isp * iden)[:, None]).reshape(NG, GR, TQ)
        phn = (en * (isn * iden)[:, None]).reshape(NG, GR, TQ)
        ph = jnp.concatenate([php, phn], axis=1).astype(bf16)

        logit = jnp.sum(xf * gw_v[...].astype(f32), axis=-1, keepdims=True)
        gate = 0.5 * jnp.tanh(0.5 * logit) + 0.5

        oT = jnp.concatenate([_dot(kvm[g], ph[g]) for g in range(NG)], axis=0)

        th = [jnp.concatenate([h_[k] for h_ in hs], axis=1) for k in range(7)]
        bs = [_strassen(th, _rhs_blocks(wd_v, c0, c0 + 128)) for c0 in range(0, HD, 128)]
        b = _block([jnp.concatenate([b_[k] for b_ in bs], axis=1) for k in range(4)])

        to = _lhs_blocks(oT[:HD, :HQ], oT[HD:, :HQ], oT[:HD, HQ:], oT[HD:, HQ:])
        for k in range(7):
            o_s[k] = to[k].T
        a = _block(_strassen([o_s[k] for k in range(7)], _rhs_blocks(wo_v, 0, HD)))

        o_v[pl.ds(r0, TQ), :] = (b + gate * (a - b)).astype(bf16)
        ocp(i).start()
        return carry

    lax.fori_loop(0, NQ, qbody, 0)
    for i in range(NQ):
        ocp(i).wait()


@jax.jit
def pallas_gated_mix__linear_kernel_hedgehog__glu_gated_bilinear__prompt_kernel(
    A_x: jax.Array,
    A_wqkv: jax.Array,
    A_w_phi: jax.Array,
    A_wo: jax.Array,
    B_x: jax.Array,
    B_w_gate: jax.Array,
    B_w_up: jax.Array,
    B_w_down: jax.Array,
    gate_w: jax.Array,
):
    del B_x
    x = A_x.reshape(S, D)
    wphi = A_w_phi.transpose(1, 2, 0).reshape(DH * DH, H)
    anyspec = pl.BlockSpec(memory_space=pl.ANY)
    out = pl.pallas_call(
        _kernel,
        in_specs=[anyspec] * 8,
        out_specs=anyspec,
        out_shape=jax.ShapeDtypeStruct((S, D), bf16),
        scratch_shapes=[
            pltpu.VMEM((S, D), bf16),
            pltpu.VMEM((D, D), bf16), pltpu.VMEM((D, D), bf16), pltpu.VMEM((D, D), bf16),
            pltpu.VMEM((DH * DH, H), bf16), pltpu.VMEM((D, D), bf16),
            pltpu.VMEM((D, F), bf16), pltpu.VMEM((D, F), bf16), pltpu.VMEM((F, D), bf16),
            pltpu.VMEM((D,), bf16),
            pltpu.VMEM((D, D), bf16), pltpu.VMEM((D, D), bf16),
            pltpu.VMEM((NG, GR, 128), bf16), pltpu.VMEM((NG, 128, 128), f32),
            pltpu.VMEM((S, D), bf16), pltpu.VMEM((7, HQ, HD), bf16),
            pltpu.SemaphoreType.DMA((10,)), pltpu.SemaphoreType.DMA((3,)),
            pltpu.SemaphoreType.DMA((NQ,)),
        ],
        compiler_params=pltpu.CompilerParams(vmem_limit_bytes=100 * 1024 * 1024),
    )(x, A_wqkv, wphi, A_wo, B_w_gate, B_w_up, B_w_down, gate_w)
    return out.reshape(1, S, D)
```
